```python
import os as _os
_os.environ.setdefault("JAX_PLATFORMS", "cpu")
import jax
import jax.numpy as jnp

def _softmax(x, axis=-1):
    return jax.nn.softmax(x, axis=axis)
def _gelu(x):
    return jax.nn.gelu(x, approximate=True)
def _silu(x):
    return jax.nn.silu(x)
def _sigmoid(x):
    return jax.nn.sigmoid(x)
def _layernorm(x, axis=-1, eps=1e-5):
    m = jnp.mean(x, axis=axis, keepdims=True)
    v = jnp.var(x, axis=axis, keepdims=True)
    return (x - m) / jnp.sqrt(v + eps)
def _scatter_add(tgt, idx, src, axis=0):
    return tgt.at[idx].add(src)
def _segment_sum(src, seg, n):
    return jax.ops.segment_sum(src, seg, n)
class _Rng:
    def __init__(self, key):
        self._k = key
    def _next(self):
        self._k, sub = jax.random.split(self._k)
        return sub
    def normal(self, shape):
        return jax.random.normal(self._next(), shape, dtype=jnp.bfloat16)
    def randint(self, lo, hi, shape):
        return jax.random.randint(self._next(), shape, lo, hi, dtype=jnp.int32)
    def uniform(self, shape, lo=0.0, hi=1.0):
        return jax.random.uniform(self._next(), shape, jnp.bfloat16, lo, hi)
    def permutation(self, n):
        return jax.random.permutation(self._next(), n)


kernel_name = 'standalone__geglu_ffn__prompt'

def setup_inputs():
    _rng = _Rng(jax.random.key(int.from_bytes(__import__("os").urandom(4), "little")))
    _w = (lambda a: (lambda t: t.astype(jnp.bfloat16) if jnp.issubdtype(t.dtype, jnp.floating) else t)(jnp.asarray(a)))
    B, S, D, F = 1, 2048, 576, 4608
    return {
        "x": _w((lambda *s: _rng.normal(s) * 0.05)(B, S, D)),
        "w_gate": _w((lambda *s: _rng.normal(s) * 0.05)(D, F)),
        "w_up": _w((lambda *s: _rng.normal(s) * 0.05)(D, F)),
        "w_down": _w((lambda *s: _rng.normal(s) * 0.05)(F, D)),
    }

def reference(x, w_gate, w_up, w_down):
    return (_gelu(x @ w_gate) * (x @ w_up)) @ w_down
```

```python
import jax
import jax.numpy as jnp
import numpy as np
from jax import lax
from jax.experimental import pallas as pl
from jax.experimental.pallas import tpu as pltpu

_C0 = float(np.sqrt(2.0 / np.pi))
_C1 = float(np.sqrt(2.0 / np.pi) * 0.044715)
_NT = (((1,), (1,)), ((), ()))

FA, TF, CM, CN, T0, T1, F0, CA = 512, 512, 512, 128, 512, 768, 256, 512


def _gelu_mul(g, u):
    t = jnp.tanh(g * (_C0 + _C1 * (g * g)))
    return (0.5 * g) * (1.0 + t) * u


@jax.jit
def pallas_standalone__geglu_ffn__prompt_kernel(x, w_gate, w_up, w_down):
    B, S, D = x.shape
    F = w_gate.shape[1]
    M = B * S
    nf = (F - FA) // TF
    assert nf * TF + FA == F and M % CM == 0 and M > T1
    f32, dt = jnp.float32, x.dtype

    def kernel(xt_hbm, wg_hbm, wu_hbm, wd_hbm, o_hbm,
               xt_v, x_v, ga, ua, da, gv, uv, dv, h_v, acc, o_v, asem, wsem, osem):
        def cp(src, dst, st, sz, sem):
            return pltpu.make_async_copy(src.at[:, pl.ds(st, sz)], dst.at[:, pl.ds(st, sz)], sem)

        grp0 = [cp(xt_hbm, xt_v, 0, T0, asem.at[0]), cp(wg_hbm, ga, 0, F0, asem.at[1]),
                cp(wu_hbm, ua, 0, F0, asem.at[2])]
        grp1 = [cp(xt_hbm, xt_v, T0, T1 - T0, asem.at[3]), cp(wg_hbm, ga, F0, FA - F0, asem.at[4]),
                cp(wu_hbm, ua, F0, FA - F0, asem.at[5])]
        grp2 = [cp(xt_hbm, xt_v, T1, M - T1, asem.at[6]), cp(wd_hbm, da, 0, FA, asem.at[7])]

        def wcp(i):
            st = FA + i * TF
            if not isinstance(i, int):
                st = pl.multiple_of(st, 128)
            return [pltpu.make_async_copy(h.at[:, pl.ds(st, TF)], v.at[i], wsem.at[k, i])
                    for k, (h, v) in enumerate(((wg_hbm, gv), (wu_hbm, uv), (wd_hbm, dv)))]

        def ocp(j):
            return cp(o_v, o_hbm, j * CN, CN, osem.at[j])

        def up(xs, wg, wu):
            g = jnp.dot(xs, wg, preferred_element_type=f32)
            u = jnp.dot(xs, wu, preferred_element_type=f32)
            return _gelu_mul(g, u).astype(dt)

        def getx(a, b):
            xs = xt_v[:, a:b].T
            x_v[a:b, :] = xs
            return xs

        for c in grp0:
            c.start()
        for c in grp0:
            c.wait()
        for c in grp1:
            c.start()
        h_v[0:T0, 0:F0] = up(getx(0, T0), ga[:, 0:F0], ua[:, 0:F0])
        for c in grp1:
            c.wait()
        for c in grp2:
            c.start()
        h_v[0:T0, F0:FA] = up(x_v[0:T0, :], ga[:, F0:FA], ua[:, F0:FA])
        h_v[T0:T1, :] = up(getx(T0, T1), ga[...], ua[...])
        for c in grp2:
            c.wait()
        for c in wcp(0):
            c.start()
        acc[:, 0:T1] = lax.dot_general(da[...], h_v[...], _NT, preferred_element_type=f32)
        a = T1
        while a < M:
            b = min(a + CA, M)
            h = up(getx(a, b), ga[...], ua[...])
            acc[:, a:b] = lax.dot_general(da[...], h, _NT, preferred_element_type=f32)
            a = b

        def body(i, carry):
            for c in wcp(i):
                c.wait()

            @pl.when(i + 1 < nf)
            def _():
                for c in wcp(i + 1):
                    c.start()

            for m in range(M // CM):
                h = up(x_v[m * CM:(m + 1) * CM, :], gv[i], uv[i])
                for j in range(CM // CN):
                    a = m * CM + j * CN
                    o = acc[:, a:a + CN] + lax.dot_general(
                        dv[i], h[j * CN:(j + 1) * CN, :], _NT, preferred_element_type=f32)
                    acc[:, a:a + CN] = o
                    o_v[:, a:a + CN] = o.astype(dt)

                    @pl.when(i == nf - 1)
                    def _():
                        ocp(a // CN).start()
            return carry

        lax.fori_loop(0, nf, body, 0)
        for j in range(M // CN):
            ocp(j).wait()

    hbm = pl.BlockSpec(memory_space=pltpu.HBM)
    V = pltpu.VMEM
    out_t = pl.pallas_call(
        kernel,
        in_specs=[hbm] * 4,
        out_specs=hbm,
        out_shape=jax.ShapeDtypeStruct((D, M), dt),
        scratch_shapes=[
            V((D, M), dt), V((M, D), dt), V((D, FA), dt), V((D, FA), dt), V((D, FA), dt),
            V((nf, D, TF), dt), V((nf, D, TF), dt), V((nf, D, TF), dt), V((T1, FA), dt),
            V((D, M), f32), V((D, M), dt),
            pltpu.SemaphoreType.DMA((8,)), pltpu.SemaphoreType.DMA((3, nf)),
            pltpu.SemaphoreType.DMA((M // CN,)),
        ],
        compiler_params=pltpu.CompilerParams(vmem_limit_bytes=100 * 2**20),
    )(x.reshape(M, D).T, w_gate, w_up, w_down.T)
    return out_t.T.reshape(B, S, D)
```

```python
import jax
import jax.numpy as jnp
import numpy as np
from jax import lax
from jax.experimental import pallas as pl
from jax.experimental.pallas import tpu as pltpu

_GELU_C0 = float(np.sqrt(2.0 / np.pi))
_GELU_C1 = float(np.sqrt(2.0 / np.pi) * 0.044715)
_NT = (((1,), (1,)), ((), ()))

_T = 128
_RAMP = ((2, 1), (3, 2), (6, 3), (16, 3))
_RAMP_REST = (("down", 0, 4), ("up", 6, 8), ("up", 8, 12), ("down", 4, 8), ("tail", 0, 8),
              ("up", 12, 16), ("down", 8, 12), ("tail", 8, 16), ("down", 12, 16))
_NH = 2
_NF = 3
_CM = 512
_VR = 16
_V0 = 64
_LAST_ROWS = 384


def _gelu_mul(g, u):
    t = jnp.tanh(g * (_GELU_C0 + _GELU_C1 * (g * g)))
    return (0.5 * g) * (1.0 + t) * u


@jax.jit
def pallas_standalone__geglu_ffn__prompt_kernel(x, w_gate, w_up, w_down):
    B, S, D = x.shape
    F = w_gate.shape[1]
    M = B * S
    f32, dt = jnp.float32, x.dtype

    ramp = [(a * _T, b * _T) for a, b in _RAMP]
    fa = ramp[-1][1]
    tf = (F - fa) // _NF
    th = M // _NH
    dm = D // _T * _T
    dr = D - dm
    assert ramp[-1][0] == M and fa + _NF * tf == F and tf % _T == 0 and th % _CM == 0
    assert 0 < dr and _LAST_ROWS < D

    def kernel(xt_hbm, wg_hbm, wu_hbm, wd_hbm, o_hbm,
               xt_v, x_v, ga, ua, da, ha, gv, uv, dv, acc, o_v, xb, wr,
               x0_sem, ramp_sem, w_sem, o_sem):

        def col_copy(src, dst, a, b, sem):
            return pltpu.make_async_copy(
                src.at[:, pl.ds(a, b - a)], dst.at[:, pl.ds(a, b - a)], sem)

        def start(copies):
            for c in copies:
                c.start()

        def wait(copies):
            for c in copies:
                c.wait()

        x0 = col_copy(xt_hbm, xt_v, 0, ramp[0][0], x0_sem)
        groups = []
        for s, (a1, b1) in enumerate(ramp):
            a0, b0 = ramp[s - 1] if s else (a1, 0)
            grp = []
            if a1 > a0:
                grp.append(col_copy(xt_hbm, xt_v, a0, a1, ramp_sem.at[s]))
            if b1 > b0:
                grp.append(col_copy(wg_hbm, ga, b0, b1, ramp_sem.at[s]))
                grp.append(col_copy(wu_hbm, ua, b0, b1, ramp_sem.at[s]))
            if s == len(ramp) - 1:
                grp.append(col_copy(wd_hbm, da, 0, fa, ramp_sem.at[s]))
            groups.append(grp)

        def w_copies(fi):
            off = fa + fi * tf
            if not isinstance(fi, int):
                off = pl.multiple_of(off, _T)
            return [pltpu.make_async_copy(src.at[:, pl.ds(off, tf)], dst.at[fi], w_sem)
                    for src, dst in ((wg_hbm, gv), (wu_hbm, uv), (wd_hbm, dv))]

        def load_x(a, b):
            xs = xt_v[:, a:b].T
            x_v[a // th, a % th:a % th + b - a, :] = xs
            return xs

        def gate_up(xs, wg, wu):
            g = jnp.dot(xs, wg, preferred_element_type=f32)
            u = jnp.dot(xs, wu, preferred_element_type=f32)
            return _gelu_mul(g, u).astype(dt)

        x0.start()
        start(groups[0] + groups[1])
        x0.wait()
        load_x(0, ramp[0][0])
        for s, (a1, b1) in enumerate(ramp[:-1]):
            wait(groups[s])
            if s + 2 < len(ramp):
                start(groups[s + 2])
            a0, b0 = ramp[s - 1] if s else (a1, 0)
            ha[0:a0, b0:b1] = gate_up(x_v[0, 0:a0, :], ga[:, b0:b1], ua[:, b0:b1])
            if a1 > a0:
                ha[a0:a1, 0:b1] = gate_up(load_x(a0, a1), ga[:, 0:b1], ua[:, 0:b1])
        wait(groups[-1])
        start(w_copies(0))
        for kind, t0, t1 in _RAMP_REST:
            a, b = t0 * _T, t1 * _T
            if kind == "up":
                ha[a:b, :] = gate_up(load_x(a, b), ga[...], ua[...])
            elif kind == "down":
                acc[a // th, :, a % th:a % th + b - a] = lax.dot_general(
                    da[...], ha[a:b, :], _NT, preferred_element_type=f32)
            else:
                for p in range(a, b, _T):
                    hf, r = p // th, p % th
                    xr = x_v[hf, r + _V0:r + _V0 + _VR, dm:D].astype(f32)
                    for k in range(dr):
                        xb[hf, r // _T, k] = jnp.broadcast_to(xr[:, k:k + 1], (_VR, _T))

        def project(hf, fi, r0, wi, w, q):
            cuts = [0]
            for p in range(0, _CM, _T):
                cuts += [p + _V0, p + _V0 + _VR]
            segs = list(zip(cuts[0::2], cuts[1::2] + [_CM]))
            main = jnp.dot(x_v[hf, r0:r0 + _CM, 0:dm], w[fi, 0:dm, q:q + _T],
                           preferred_element_type=f32)
            x_rem = jnp.concatenate([x_v[hf, r0 + a:r0 + b, dm:D] for a, b in segs], axis=0)
            rem = jnp.dot(x_rem, w[fi, dm:D, q:q + _T], preferred_element_type=f32)
            parts, o = [], 0
            for n, (a, b) in enumerate(segs):
                parts.append(rem[o:o + b - a])
                o += b - a
                if n + 1 < len(segs):
                    tot = None
                    for k in range(dr):
                        term = xb[hf, r0 // _T + n, k] * jnp.broadcast_to(
                            wr[wi, k:k + 1, q:q + _T], (_VR, _T))
                        tot = term if tot is None else tot + term
                    parts.append(tot)
            return main + jnp.concatenate(parts, axis=0)

        def step(i, carry):
            fi, hf = i // _NH, i % _NH

            @pl.when(hf == 0)
            def _():
                wait(w_copies(fi))

            wr[0] = gv[fi, dm:D, :].astype(f32)
            wr[1] = uv[fi, dm:D, :].astype(f32)
            for r0 in range(0, th, _CM):
                h = jnp.concatenate(
                    [_gelu_mul(project(hf, fi, r0, 0, gv, q),
                               project(hf, fi, r0, 1, uv, q)).astype(dt)
                     for q in range(0, tf, _T)], axis=1)
                if r0 == 0:
                    @pl.when(jnp.logical_and(hf == 0, fi + 1 < _NF))
                    def _():
                        start(w_copies(jnp.minimum(fi + 1, _NF - 1)))

                for j in range(0, _CM, _T):
                    a = r0 + j
                    rows = ((0, _LAST_ROWS), (_LAST_ROWS, D)) if a + _T == th else ((0, D),)
                    for d0, d1 in rows:
                        o = acc[hf, d0:d1, a:a + _T] + lax.dot_general(
                            dv[fi, d0:d1, :], h[j:j + _T, :], _NT, preferred_element_type=f32)
                        acc[hf, d0:d1, a:a + _T] = o
                        o_v[hf, d0:d1, a:a + _T] = o.astype(dt)

                        @pl.when(fi == _NF - 1)
                        def _():
                            col = pl.multiple_of(hf * th + a, _T)
                            pltpu.make_async_copy(
                                o_v.at[hf, pl.ds(d0, d1 - d0), pl.ds(a, _T)],
                                o_hbm.at[pl.ds(d0, d1 - d0), pl.ds(col, _T)], o_sem).start()
            return carry

        lax.fori_loop(0, _NF * _NH, step, 0)
        pltpu.make_async_copy(o_v, o_v, o_sem).wait()

    hbm = pl.BlockSpec(memory_space=pltpu.HBM)
    vmem, sem = pltpu.VMEM, pltpu.SemaphoreType.DMA
    out_t = pl.pallas_call(
        kernel,
        in_specs=[hbm] * 4,
        out_specs=hbm,
        out_shape=jax.ShapeDtypeStruct((D, M), dt),
        scratch_shapes=[
            vmem((D, M), dt),
            vmem((_NH, th, D), dt),
            vmem((D, fa), dt), vmem((D, fa), dt), vmem((D, fa), dt),
            vmem((M, fa), dt),
            vmem((_NF, D, tf), dt), vmem((_NF, D, tf), dt), vmem((_NF, D, tf), dt),
            vmem((_NH, D, th), f32),
            vmem((_NH, D, th), dt),
            vmem((_NH, th // _T, dr, _VR, _T), f32),
            vmem((2, dr, tf), f32),
            sem(()), sem((len(ramp),)), sem(()), sem(()),
        ],
        compiler_params=pltpu.CompilerParams(
            vmem_limit_bytes=100 * 2**20,
            disable_bounds_checks=True,
            disable_semaphore_checks=True,
        ),
    )(x.reshape(M, D).T, w_gate, w_up, w_down.T)
    return out_t.T.reshape(B, S, D)
```

```python
import jax
import jax.numpy as jnp
import numpy as np
from jax import lax
from jax.experimental import pallas as pl
from jax.experimental.pallas import tpu as pltpu

_GELU_C0 = float(np.sqrt(2.0 / np.pi))
_GELU_C1 = float(np.sqrt(2.0 / np.pi) * 0.044715)
_NT = (((1,), (1,)), ((), ()))

_T = 128
_RAMP = ((2, 1), (3, 2), (6, 3), (16, 3))
_RAMP_REST = (("down", 0, 4), ("up", 6, 8), ("up", 8, 12), ("down", 4, 8), ("tail", 0, 8),
              ("up", 12, 16), ("down", 8, 12), ("tail", 8, 16), ("down", 12, 16))
_NH = 2
_NF = 3
_CM = 512
_VR = 16
_V0 = 64
_LAST_ROWS = 384


def _gelu_mul(g, u):
    t = jnp.tanh(g * (_GELU_C0 + _GELU_C1 * (g * g)))
    return (0.5 * g) * (1.0 + t) * u


@jax.jit
def pallas_standalone__geglu_ffn__prompt_kernel(x, w_gate, w_up, w_down):
    B, S, D = x.shape
    F = w_gate.shape[1]
    M = B * S
    f32, dt = jnp.float32, x.dtype

    ramp = [(a * _T, b * _T) for a, b in _RAMP]
    fa = ramp[-1][1]
    tf = (F - fa) // _NF
    th = M // _NH
    dm = D // _T * _T
    dr = D - dm
    assert ramp[-1][0] == M and fa + _NF * tf == F and tf % _T == 0 and th % _CM == 0
    assert 0 < dr and _LAST_ROWS < D

    def kernel(xt_hbm, wg_hbm, wu_hbm, wd_hbm, o_hbm,
               xt_v, x_v, ga, ua, da, ha, gv, uv, dv, acc, o_v, xb, wr,
               x0_sem, ramp_sem, w_sem, o_sem):

        def col_copy(src, dst, a, b, sem):
            return pltpu.make_async_copy(
                src.at[:, pl.ds(a, b - a)], dst.at[:, pl.ds(a, b - a)], sem)

        def start(copies):
            for c in copies:
                c.start()

        def wait(copies):
            for c in copies:
                c.wait()

        x0 = col_copy(xt_hbm, xt_v, 0, ramp[0][0], x0_sem)
        groups = []
        for s, (a1, b1) in enumerate(ramp):
            a0, b0 = ramp[s - 1] if s else (a1, 0)
            grp = []
            if a1 > a0:
                grp.append(col_copy(xt_hbm, xt_v, a0, a1, ramp_sem.at[s]))
            if b1 > b0:
                grp.append(col_copy(wg_hbm, ga, b0, b1, ramp_sem.at[s]))
                grp.append(col_copy(wu_hbm, ua, b0, b1, ramp_sem.at[s]))
            if s == len(ramp) - 1:
                grp.append(col_copy(wd_hbm, da, 0, fa, ramp_sem.at[s]))
            groups.append(grp)

        def w_copies(fi):
            off = fa + fi * tf
            if not isinstance(fi, int):
                off = pl.multiple_of(off, _T)
            return [pltpu.make_async_copy(src.at[:, pl.ds(off, tf)], dst.at[fi], w_sem)
                    for src, dst in ((wg_hbm, gv), (wu_hbm, uv), (wd_hbm, dv))]

        def load_x(a, b):
            xs = xt_v[:, a:b].T
            x_v[a // th, a % th:a % th + b - a, :] = xs
            return xs

        def gate_up(xs, wg, wu):
            g = jnp.dot(xs, wg, preferred_element_type=f32)
            u = jnp.dot(xs, wu, preferred_element_type=f32)
            return _gelu_mul(g, u).astype(dt)

        x0.start()
        start(groups[0] + groups[1])
        x0.wait()
        load_x(0, ramp[0][0])
        for s, (a1, b1) in enumerate(ramp[:-1]):
            wait(groups[s])
            if s + 2 < len(ramp):
                start(groups[s + 2])
            a0, b0 = ramp[s - 1] if s else (a1, 0)
            ha[0:a0, b0:b1] = gate_up(x_v[0, 0:a0, :], ga[:, b0:b1], ua[:, b0:b1])
            if a1 > a0:
                ha[a0:a1, 0:b1] = gate_up(load_x(a0, a1), ga[:, 0:b1], ua[:, 0:b1])
        wait(groups[-1])
        start(w_copies(0))
        for kind, t0, t1 in _RAMP_REST:
            a, b = t0 * _T, t1 * _T
            if kind == "up":
                ha[a:b, :] = gate_up(load_x(a, b), ga[...], ua[...])
            elif kind == "down":
                acc[a // th, :, a % th:a % th + b - a] = lax.dot_general(
                    da[...], ha[a:b, :], _NT, preferred_element_type=f32)
            else:
                for p in range(a, b, _T):
                    hf, r = p // th, p % th
                    xr = x_v[hf, r + _V0:r + _V0 + _VR, dm:D].astype(f32)
                    for k in range(dr):
                        xb[hf, r // _T, k] = jnp.broadcast_to(xr[:, k:k + 1], (_VR, _T))

        def project(hf, fi, r0, wi, w, q):
            cuts = [0]
            for p in range(0, _CM, _T):
                cuts += [p + _V0, p + _V0 + _VR]
            segs = list(zip(cuts[0::2], cuts[1::2] + [_CM]))
            main = jnp.dot(x_v[hf, r0:r0 + _CM, 0:dm], w[fi, 0:dm, q:q + _T],
                           preferred_element_type=f32)
            x_rem = jnp.concatenate([x_v[hf, r0 + a:r0 + b, dm:D] for a, b in segs], axis=0)
            rem = jnp.dot(x_rem, w[fi, dm:D, q:q + _T], preferred_element_type=f32)
            w_rows = [jnp.broadcast_to(wr[wi, k:k + 1, q:q + _T], (_VR, _T)) for k in range(dr)]
            parts, o = [], 0
            for n, (a, b) in enumerate(segs):
                parts.append(rem[o:o + b - a])
                o += b - a
                if n + 1 < len(segs):
                    x_cols = xb[hf, r0 // _T + n]
                    tot = x_cols[0] * w_rows[0]
                    for k in range(1, dr):
                        tot = tot + x_cols[k] * w_rows[k]
                    parts.append(tot)
            return main + jnp.concatenate(parts, axis=0)

        def step(i, carry):
            fi, hf = i // _NH, i % _NH

            @pl.when(hf == 0)
            def _():
                wait(w_copies(fi))

            wr[0] = gv[fi, dm:D, :].astype(f32)
            wr[1] = uv[fi, dm:D, :].astype(f32)
            for r0 in range(0, th, _CM):
                h = jnp.concatenate(
                    [_gelu_mul(project(hf, fi, r0, 0, gv, q),
                               project(hf, fi, r0, 1, uv, q)).astype(dt)
                     for q in range(0, tf, _T)], axis=1)
                if r0 == 0:
                    @pl.when(jnp.logical_and(hf == 0, fi + 1 < _NF))
                    def _():
                        start(w_copies(jnp.minimum(fi + 1, _NF - 1)))

                for j in range(0, _CM, _T):
                    a = r0 + j
                    rows = ((0, _LAST_ROWS), (_LAST_ROWS, D)) if a + _T == th else ((0, D),)
                    for d0, d1 in rows:
                        o = acc[hf, d0:d1, a:a + _T] + lax.dot_general(
                            dv[fi, d0:d1, :], h[j:j + _T, :], _NT, preferred_element_type=f32)
                        acc[hf, d0:d1, a:a + _T] = o
                        o_v[hf, d0:d1, a:a + _T] = o.astype(dt)

                        @pl.when(fi == _NF - 1)
                        def _():
                            col = pl.multiple_of(hf * th + a, _T)
                            pltpu.make_async_copy(
                                o_v.at[hf, pl.ds(d0, d1 - d0), pl.ds(a, _T)],
                                o_hbm.at[pl.ds(d0, d1 - d0), pl.ds(col, _T)], o_sem).start()
            return carry

        lax.fori_loop(0, _NF * _NH, step, 0)
        pltpu.make_async_copy(o_v, o_v, o_sem).wait()

    hbm = pl.BlockSpec(memory_space=pltpu.HBM)
    vmem, sem = pltpu.VMEM, pltpu.SemaphoreType.DMA
    out_t = pl.pallas_call(
        kernel,
        in_specs=[hbm] * 4,
        out_specs=hbm,
        out_shape=jax.ShapeDtypeStruct((D, M), dt),
        scratch_shapes=[
            vmem((D, M), dt),
            vmem((_NH, th, D), dt),
            vmem((D, fa), dt), vmem((D, fa), dt), vmem((D, fa), dt),
            vmem((M, fa), dt),
            vmem((_NF, D, tf), dt), vmem((_NF, D, tf), dt), vmem((_NF, D, tf), dt),
            vmem((_NH, D, th), f32),
            vmem((_NH, D, th), dt),
            vmem((_NH, th // _T, dr, _VR, _T), f32),
            vmem((2, dr, tf), f32),
            sem(()), sem((len(ramp),)), sem(()), sem(()),
        ],
        compiler_params=pltpu.CompilerParams(
            vmem_limit_bytes=100 * 2**20,
            disable_bounds_checks=True,
            disable_semaphore_checks=True,
        ),
    )(x.reshape(M, D).T, w_gate, w_up, w_down.T)
    return out_t.T.reshape(B, S, D)
```
